```python
import os as _os
_os.environ.setdefault("JAX_PLATFORMS", "cpu")
import jax
import jax.numpy as jnp

def _softmax(x, axis=-1):
    return jax.nn.softmax(x, axis=axis)
def _gelu(x):
    return jax.nn.gelu(x, approximate=True)
def _silu(x):
    return jax.nn.silu(x)
def _sigmoid(x):
    return jax.nn.sigmoid(x)
def _layernorm(x, axis=-1, eps=1e-5):
    m = jnp.mean(x, axis=axis, keepdims=True)
    v = jnp.var(x, axis=axis, keepdims=True)
    return (x - m) / jnp.sqrt(v + eps)
def _scatter_add(tgt, idx, src, axis=0):
    return tgt.at[idx].add(src)
def _segment_sum(src, seg, n):
    return jax.ops.segment_sum(src, seg, n)
class _Rng:
    def __init__(self, key):
        self._k = key
    def _next(self):
        self._k, sub = jax.random.split(self._k)
        return sub
    def normal(self, shape):
        return jax.random.normal(self._next(), shape, dtype=jnp.bfloat16)
    def randint(self, lo, hi, shape):
        return jax.random.randint(self._next(), shape, lo, hi, dtype=jnp.int32)
    def uniform(self, shape, lo=0.0, hi=1.0):
        return jax.random.uniform(self._next(), shape, jnp.bfloat16, lo, hi)
    def permutation(self, n):
        return jax.random.permutation(self._next(), n)


kernel_name = 'concat_heads__mha_block__linear_attn_block__prompt'

def setup_inputs():
    _rng = _Rng(jax.random.key(int.from_bytes(__import__("os").urandom(4), "little")))
    _w = (lambda a: (lambda t: t.astype(jnp.bfloat16) if jnp.issubdtype(t.dtype, jnp.floating) else t)(jnp.asarray(a)))
    def _A_setup():
        B, S, D, H = 1, 2048, 1024, 32
        return {
            "x": _w((lambda *s: _rng.normal(s) * 0.2)(B, S, D)),
            "wqkv": _w((lambda *s: _rng.normal(s) * 0.2)(D, 3 * D)),
            "wo": _w((lambda *s: _rng.normal(s) * 0.05)(D, D)),
        }
    _A_in = _A_setup()

    def _B_setup():
        B, S, D = 1, 2048, 1024
        return {
            "x": _w((lambda *s: _rng.normal(s) * 0.05)(B, S, D)),
            "wqkv": _w((lambda *s: _rng.normal(s) * 1.6)(D, 3 * D)),
            "wo": _w((lambda *s: _rng.normal(s) * 0.1)(D, D)),
        }
    _B_in = _B_setup()

    return {
        "A_x": _A_in["x"],
        "A_wqkv": _A_in["wqkv"],
        "A_wo": _A_in["wo"],
        "B_x": _B_in["x"],
        "B_wqkv": _B_in["wqkv"],
        "B_wo": _B_in["wo"],
    }

def reference(A_x, A_wqkv, A_wo, B_x, B_wqkv, B_wo):
    def _A_ref(x, wqkv, wo):
        B, S, D = x.shape
        H = 32
        Dh = D // H
        qkv = (lambda x, *d: x.transpose(*d))((x @ wqkv).reshape(B, S, 3, H, Dh), 2, 0, 3, 1, 4)
        q, k, v = qkv[0], qkv[1], qkv[2]
        scores = jnp.einsum("bhqd,bhkd->bhqk", q, k) * (Dh ** -0.5)
        p = _softmax(scores, axis=-1)
        o = jnp.einsum("bhqk,bhkd->bhqd", p, v)
        return (lambda x, *d: x.transpose(*d))(o, 0, 2, 1, 3).reshape(B, S, D) @ wo

    def _B_ref(x, wqkv, wo):
        B, S, D = x.shape
        H = 32; Dh = D // H
        qkv = (lambda x, *d: x.transpose(*d))((x @ wqkv).reshape(B, S, 3, H, Dh), 2, 0, 3, 1, 4)
        q, k, v = qkv[0], qkv[1], qkv[2]
        phi = lambda t: jnp.where(t > 0, t + 1, jnp.exp(t)) + 1e-6
        pq, pk = phi(q), phi(k)
        kv = jnp.einsum("bhsd,bhse->bhde", pk, v)
        z = jnp.einsum("bhsd->bhd", pk)
        num = jnp.einsum("bhqd,bhde->bhqe", pq, kv)
        den = jnp.einsum("bhqd,bhd->bhq", pq, z)[..., None] + 1e-6
        o = num / den
        return (lambda x, *d: x.transpose(*d))(o, 0, 2, 1, 3).reshape(B, S, D) @ wo

    a = _A_ref(A_x, A_wqkv, A_wo)
    b = _B_ref(B_x, B_wqkv, B_wo)
    return jnp.concatenate([a, b], axis=-1)
```

```python
import functools
import math

import jax
import jax.numpy as jnp
import jax.experimental.pallas as pl
import jax.experimental.pallas.tpu as pltpu

S = 2048
D = 1024
H = 32
DH = 32
G = 8
HG = 4

TR = 512
NR = S // TR
TQ = 512
NQ = S // TQ
CK = 128
NC = S // CK
NT = H * NQ
LAG = 3

F32 = jnp.float32
BF16 = jnp.bfloat16

QSCALE = (DH ** -0.5) * math.log2(math.e)


def _tie(x, dep):
    b = jax.lax.bitcast_convert_type(dep, jnp.int32)
    return jnp.where((b | 1) == 0, jnp.zeros_like(x), x)


def _phi(t):
    return jnp.where(t > 0, t + 1.0, jnp.exp(jnp.minimum(t, 0.0))) + 1e-6


def _kernel(xa_hbm, wa_hbm, woa_hbm, xb_hbm, wb_hbm, wob_hbm, out_hbm,
            xa, wa, woa, xb, wb, wob,
            qt, vt, kh, s0, s1, otb, oa,
            pq, pkt, vb, zacc, zd, mm,
            stage, in_sems, out_sems):
    copies = [
        pltpu.make_async_copy(xa_hbm, xa, in_sems.at[0]),
        pltpu.make_async_copy(wa_hbm, wa, in_sems.at[1]),
        pltpu.make_async_copy(xb_hbm, xb, in_sems.at[2]),
        pltpu.make_async_copy(wb_hbm, wb, in_sems.at[3]),
        pltpu.make_async_copy(woa_hbm, woa, in_sems.at[4]),
        pltpu.make_async_copy(wob_hbm, wob, in_sems.at[5]),
    ]
    for c in copies:
        c.start()

    def out_copy(slot, r, col):
        return pltpu.make_async_copy(
            stage.at[slot],
            out_hbm.at[pl.ds(r * TR, TR), pl.ds(col * D, D)],
            out_sems.at[slot])

    copies[0].wait()
    copies[1].wait()

    def a_proj(r, carry):
        rows = pl.ds(pl.multiple_of(r * TR, TR), TR)
        x = xa[rows, :]
        for c in range(2):
            y = jnp.dot(x, wa[:, c * 512:(c + 1) * 512], preferred_element_type=F32)
            qt[c * 512:(c + 1) * 512, rows] = (y * QSCALE).T.astype(BF16)
        for c in range(2):
            y = jnp.dot(x, wa[:, D + c * 512:D + (c + 1) * 512], preferred_element_type=F32)
            for hh in range(16):
                kh[c * 16 + hh, rows, :] = y[:, hh * DH:(hh + 1) * DH].astype(BF16)
        for c in range(2):
            y = jnp.dot(x, wa[:, 2 * D + c * 512:2 * D + (c + 1) * 512], preferred_element_type=F32)
            vt[c * 512:(c + 1) * 512, rows] = y.T.astype(BF16)
        return carry

    jax.lax.fori_loop(0, NR, a_proj, 0)

    sbuf = [s0, s1]

    def hj(t):
        blk = t // HG
        g = blk // NQ
        j = blk % NQ
        return g * HG + t % HG, j

    def stage_fn(t_qk, s_w, t_sm, u_sm, s_r, m_sm, off, do_sm=True):
        h1, j1 = hj(t_qk)
        q = qt[pl.ds(pl.multiple_of(h1 * DH, DH), DH), pl.ds(pl.multiple_of(j1 * TQ, TQ), TQ)]
        if do_sm:
            h0, _ = hj(t_sm)
            mb = jnp.broadcast_to(m_sm, (8, TQ))
        m8 = None
        l8 = None
        acc = None
        hist = []
        for c in range(NC):
            s = jnp.dot(kh[h1, c * CK:(c + 1) * CK, :], q, preferred_element_type=F32)
            s_w[c * CK:(c + 1) * CK, :] = s
            s3 = s.reshape(CK // 8, 8, TQ)
            for r in range(CK // 8):
                m8 = s3[r] if m8 is None else jnp.maximum(m8, s3[r])
            hist.append(m8)
            if do_sm:
                mbc = _tie(mb, hist[c - LAG]) if c >= LAG else mb
                sv = s_r[pl.ds(pl.multiple_of(off + c * CK, 8), CK), :]
                p = jnp.exp2(sv.reshape(CK // 8, 8, TQ) - mbc[None])
                for kt in range(CK // 128):
                    lt = None
                    for r in reversed(range(16)):
                        x = p[kt * 16 + r]
                        lt = x if lt is None else lt + x
                    l8 = lt if l8 is None else l8 + lt
                v = vt[pl.ds(pl.multiple_of(h0 * DH, DH), DH), c * CK:(c + 1) * CK]
                o = jnp.dot(v, p.reshape(CK, TQ).astype(BF16), preferred_element_type=F32)
                acc = o if acc is None else acc + o
        if do_sm:
            l = jnp.sum(l8, axis=0, keepdims=True)
            otb[u_sm * DH:(u_sm + 1) * DH, :] = acc / l
        return jnp.max(m8, axis=0, keepdims=True)

    def flush_o(blk):
        g = blk // NQ
        j = blk % NQ
        oa[pl.ds(pl.multiple_of(j * TQ, TQ), TQ), pl.ds(pl.multiple_of(g * 128, 128), 128)] = (
            otb[...].T.astype(BF16))

    m_init = stage_fn(0, s0, None, None, None, None, None, do_sm=False)

    def attn_body(i, m):
        t = i * HG
        off = (i >> 20) * 8
        for u in range(HG):
            m = stage_fn(jnp.minimum(t + u + 1, NT - 1), sbuf[(u + 1) % 2], t + u, u, sbuf[u % 2], m, off)
        flush_o(i)
        return m

    jax.lax.fori_loop(0, NT // HG, attn_body, m_init)

    copies[4].wait()

    def a_out(r, carry):
        slot = r % 2

        @pl.when(r >= 2)
        def _():
            out_copy(slot, r - 2, 0).wait()

        rows = pl.ds(pl.multiple_of(r * TR, TR), TR)
        y = jnp.dot(oa[rows, :], woa[...], preferred_element_type=F32)
        stage[slot] = y.astype(BF16)
        out_copy(slot, r, 0).start()
        return carry

    jax.lax.fori_loop(0, NR, a_out, 0)

    copies[2].wait()
    copies[3].wait()
    zacc[...] = jnp.zeros_like(zacc)

    def b_proj(r, carry):
        rows = pl.ds(pl.multiple_of(r * TR, TR), TR)
        x = xb[rows, :]
        for c in range(2):
            y = jnp.dot(x, wb[:, c * 512:(c + 1) * 512], preferred_element_type=F32)
            pq[rows, c * 512:(c + 1) * 512] = _phi(y).astype(BF16)
        for c in range(2):
            y = jnp.dot(x, wb[:, D + c * 512:D + (c + 1) * 512], preferred_element_type=F32)
            pk = _phi(y)
            zacc[:, c * 512:(c + 1) * 512] += jnp.sum(pk.reshape(TR // 8, 8, 512), axis=0)
            pkt[c * 512:(c + 1) * 512, rows] = pk.T.astype(BF16)
        for c in range(2):
            y = jnp.dot(x, wb[:, 2 * D + c * 512:2 * D + (c + 1) * 512], preferred_element_type=F32)
            vb[rows, c * 512:(c + 1) * 512] = y.astype(BF16)
        return carry

    jax.lax.fori_loop(0, NR, b_proj, 0)

    copies[5].wait()
    rh = jax.lax.broadcasted_iota(jnp.int32, (128, 128), 0) // DH
    ch = jax.lax.broadcasted_iota(jnp.int32, (128, 128), 1) // DH
    same_head = rh == ch
    z = jnp.sum(zacc[...], axis=0, keepdims=True)
    for g in range(G):
        sl = slice(g * 128, (g + 1) * 128)
        kv = jnp.dot(pkt[sl, :], vb[:, sl], preferred_element_type=F32)
        kvd = jnp.where(same_head, kv, 0.0).astype(BF16)
        mm[sl, :] = jnp.dot(kvd, wob[sl, :], preferred_element_type=F32).astype(BF16)
        zc = jnp.broadcast_to(z[:, sl], (128, 128)).T
        zd[g] = jnp.where(same_head, zc, 0.0).astype(BF16)

    def b_out(r, carry):
        slot = r % 2

        @pl.when(r < 2)
        def _():
            out_copy(slot, NR - 2 + r, 0).wait()

        @pl.when(r >= 2)
        def _():
            out_copy(slot, r - 2, 1).wait()

        rows = pl.ds(pl.multiple_of(r * TR, TR), TR)
        parts = []
        for g in range(G):
            a = pq[rows, g * 128:(g + 1) * 128]
            den = jnp.dot(a, zd[g], preferred_element_type=F32) + 1e-6
            parts.append((a.astype(F32) / den).astype(BF16))
        an = jnp.concatenate(parts, axis=1)
        y = jnp.dot(an, mm[...], preferred_element_type=F32)
        stage[slot] = y.astype(BF16)
        out_copy(slot, r, 1).start()
        return carry

    jax.lax.fori_loop(0, NR, b_out, 0)
    out_copy(0, NR - 2, 1).wait()
    out_copy(1, NR - 1, 1).wait()


@jax.jit
def pallas_concat_heads__mha_block__linear_attn_block__prompt_kernel(
    A_x: jax.Array,
    A_wqkv: jax.Array,
    A_wo: jax.Array,
    B_x: jax.Array,
    B_wqkv: jax.Array,
    B_wo: jax.Array,
):
    xa = A_x.reshape(S, D)
    xb = B_x.reshape(S, D)
    any_spec = pl.BlockSpec(memory_space=pl.ANY)
    out = pl.pallas_call(
        _kernel,
        out_shape=jax.ShapeDtypeStruct((S, 2 * D), BF16),
        in_specs=[any_spec] * 6,
        out_specs=any_spec,
        scratch_shapes=[
            pltpu.VMEM((S, D), BF16),
            pltpu.VMEM((D, 3 * D), BF16),
            pltpu.VMEM((D, D), BF16),
            pltpu.VMEM((S, D), BF16),
            pltpu.VMEM((D, 3 * D), BF16),
            pltpu.VMEM((D, D), BF16),
            pltpu.VMEM((D, S), BF16),
            pltpu.VMEM((D, S), BF16),
            pltpu.VMEM((H, S, DH), BF16),
            pltpu.VMEM((S, TQ), F32),
            pltpu.VMEM((S, TQ), F32),
            pltpu.VMEM((128, TQ), F32),
            pltpu.VMEM((S, D), BF16),
            pltpu.VMEM((S, D), BF16),
            pltpu.VMEM((D, S), BF16),
            pltpu.VMEM((S, D), BF16),
            pltpu.VMEM((8, D), F32),
            pltpu.VMEM((G, 128, 128), BF16),
            pltpu.VMEM((D, D), BF16),
            pltpu.VMEM((2, TR, D), BF16),
            pltpu.SemaphoreType.DMA((6,)),
            pltpu.SemaphoreType.DMA((2,)),
        ],
        compiler_params=pltpu.CompilerParams(vmem_limit_bytes=120 * 1024 * 1024),
    )(xa, A_wqkv, A_wo, xb, B_wqkv, B_wo)
    return out.reshape(1, S, 2 * D)
```

```python
import math

import jax
import jax.numpy as jnp
import jax.experimental.pallas as pl
import jax.experimental.pallas.tpu as pltpu

S = 2048
D = 1024
H = 32
DH = 32
G = 8

TR = 512
NR = S // TR
CW = 512
XP = 256
WP = 256
TQ = 512
NQ = S // TQ
CK = 128
NC = S // CK
NT = H * NQ
TPI = 8
NBUF = 4
SK = 1
LAG = 3

F32 = jnp.float32
BF16 = jnp.bfloat16
U32 = jnp.uint32

QSCALE = (DH ** -0.5) * math.log2(math.e)


def _tie(x, dep):
    b = jax.lax.bitcast_convert_type(dep, jnp.int32)
    return jnp.where((b | 1) == 0, jnp.zeros_like(x), x)


def _phi(t):
    return jnp.where(t > 0, t + 1.0, jnp.exp(jnp.minimum(t, 0.0))) + 1e-6


def _pack(x):
    return pltpu.bitcast(x.astype(BF16), U32)


def _unpack(x):
    return pltpu.bitcast(x, BF16)


def _recip(x):
    r = pl.reciprocal(x, approx=True)
    return r * (2.0 - x * r)


def _kernel(xa_hbm, wa_hbm, woa_hbm, xb_hbm, wb_hbm, wob_hbm, out_hbm,
            xa, wa, woa, xb, wb, wob,
            qt, vt, kh, sb0, sb1, sb2, sb3, ot,
            pq, kvacc, zacc, mm, an,
            stage, stageb, xa_sems, wa_sems, in_sems, out_sems, outb_sems):
    def xa_copy(p):
        rows = pl.ds(p * XP, XP)
        return pltpu.make_async_copy(xa_hbm.at[rows, :], xa.at[rows, :], xa_sems.at[p])

    def wa_copy(p):
        cols = pl.ds(p * WP, WP)
        return pltpu.make_async_copy(wa_hbm.at[:, cols], wa.at[:, cols], wa_sems.at[p])

    rest = []
    rest_all = []
    for b, (src, dst, nrows) in enumerate(
            ((woa_hbm, woa, 512), (wb_hbm, wb, 176), (xb_hbm, xb, 512), (wob_hbm, wob, 512))):
        n = src.shape[0]
        r0 = 0
        while r0 < n:
            nr = min(nrows, n - r0)
            rest.append(pltpu.make_async_copy(src.at[pl.ds(r0, nr), :], dst.at[pl.ds(r0, nr), :],
                                              in_sems.at[b]))
            r0 += nr
        rest_all.append(pltpu.make_async_copy(src, dst, in_sems.at[b]))

    def out_copy(slot, r, col):
        return pltpu.make_async_copy(
            stage.at[slot],
            out_hbm.at[pl.ds(r * TR, TR), pl.ds(col * D, D)],
            out_sems.at[slot])

    def a_proj_piece(r0, nr, c0, nc):
        static = isinstance(r0, int)
        rows = pl.ds(r0 if static else pl.multiple_of(r0, nr), nr)
        rows2 = pl.ds(r0 // 2 if static else pl.multiple_of(r0 // 2, nr // 2), nr // 2)
        y = jnp.dot(xa[rows, :], wa[:, c0:c0 + nc], preferred_element_type=F32)
        f0 = c0 % D
        if c0 < D:
            qt[f0 // 2:(f0 + nc) // 2, rows] = _pack((y * QSCALE).T)
        elif c0 < 2 * D:
            for hh in range(nc // DH):
                kh[f0 // DH + hh, rows2, :] = _pack(y[:, hh * DH:(hh + 1) * DH])
        else:
            vt[f0 // 2:(f0 + nc) // 2, rows] = _pack(y.T)

    xa_copy(0).start()
    wa_copy(0).start()
    sb2[...] = jnp.zeros_like(sb2)
    sb3[...] = jnp.zeros_like(sb3)
    zacc[...] = jnp.zeros_like(zacc)
    kvacc[...] = jnp.zeros_like(kvacc)
    xa_copy(0).wait()
    wa_copy(1).start()
    wa_copy(0).wait()
    xa_copy(1).start()
    a_proj_piece(0, 256, 0, 256)
    wa_copy(1).wait()
    wa_copy(2).start()
    wa_copy(3).start()
    a_proj_piece(0, 256, 256, 256)
    xa_copy(1).wait()
    wa_copy(4).start()
    a_proj_piece(256, 256, 0, 512)
    wa_copy(2).wait()
    wa_copy(3).wait()
    for p in (5, 6, 7):
        wa_copy(p).start()
    a_proj_piece(0, 512, 512, 512)
    for p in (4, 5, 6, 7):
        wa_copy(p).wait()
    for p in (8, 9, 10, 11):
        wa_copy(p).start()
    a_proj_piece(0, 512, 1024, 512)
    a_proj_piece(0, 512, 1536, 512)
    for p in (8, 9, 10, 11):
        wa_copy(p).wait()
    xa_copy(2).start()
    xa_copy(3).start()
    a_proj_piece(0, 512, 2048, 512)
    a_proj_piece(0, 512, 2560, 512)

    def a_proj(r, carry):
        xa_copy(2 * r).wait()
        xa_copy(2 * r + 1).wait()

        @pl.when(r + 1 < NR)
        def _():
            xa_copy(2 * r + 2).start()
            xa_copy(2 * r + 3).start()

        for c in range(6):
            a_proj_piece(r * TR, TR, c * CW, CW)
        return carry

    jax.lax.fori_loop(1, NR, a_proj, 0)

    sbuf = [sb0, sb1, sb2, sb3]

    def hj(t):
        return t // NQ, t % NQ

    def load_q(t):
        h1, j1 = hj(t)
        q = qt[pl.ds(pl.multiple_of(h1 * (DH // 2), DH // 2), DH // 2),
               pl.ds(pl.multiple_of(j1 * TQ, TQ), TQ)]
        return h1, _unpack(q)

    def qk_chunk(h1, q, c, s_w, m8):
        k = _unpack(kh[h1, c * (CK // 2):(c + 1) * (CK // 2), :])
        s = jnp.dot(k, q, preferred_element_type=F32)
        s_w[c * CK:(c + 1) * CK, :] = s
        s3 = s.reshape(CK // 8, 8, TQ)
        for r in range(CK // 8):
            m8 = s3[r] if m8 is None else jnp.maximum(m8, s3[r])
        return m8

    def sm_chunk(h0, c, s_r, mbc, off, l8, acc):
        sv = s_r[pl.ds(pl.multiple_of(off + c * CK, 8), CK), :].reshape(CK // 8, 8, TQ)
        ps = [None] * (CK // 8)
        lt = None
        for r in reversed(range(CK // 8)):
            x = jnp.exp2(sv[r] - mbc)
            ps[r] = x
            lt = x if lt is None else lt + x
        l8 = lt if l8 is None else l8 + lt
        p = jnp.concatenate(ps, axis=0).astype(BF16)
        v = _unpack(vt[pl.ds(pl.multiple_of(h0 * (DH // 2), DH // 2), DH // 2), c * CK:(c + 1) * CK])
        o = jnp.dot(v, p, preferred_element_type=F32)
        acc = o if acc is None else acc + o
        return l8, acc

    def colmax(m8):
        return jnp.broadcast_to(jnp.max(m8, axis=0, keepdims=True), (8, TQ))

    def finish(t, l8, acc):
        h0, j0 = hj(jnp.maximum(t, 0))
        l = jnp.sum(l8, axis=0, keepdims=True)
        ot[pl.ds(pl.multiple_of(h0 * DH, DH), DH), pl.ds(pl.multiple_of(j0 * TQ, TQ), TQ)] = (
            acc * _recip(l)).astype(BF16)

    def attn_body(i, carry):
        mb, l8, acc, mb_next = carry
        for n, cp in enumerate(rest):
            @pl.when(i == n + 1)
            def _():
                cp.start()
        t0 = i * TPI
        off = (i >> 20) * 8
        hist = []
        h0, _ = hj(jnp.maximum(t0 - 2, 0))
        for u in range(TPI):
            h1, q = load_q(t0 + u)
            m8 = None
            for c in range(NC):
                m8 = qk_chunk(h1, q, c, sbuf[u % NBUF], m8)
                hist.append(m8)
                us = u - 1 if c >= SK else u - 2
                cs = (c - SK) % NC
                if cs == 0:
                    h0, _ = hj(jnp.maximum(t0 + us, 0))
                    mb, l8, acc = mb_next, None, None
                k = len(hist) - 1 - LAG
                mbc = _tie(mb, hist[k]) if k >= 0 else mb
                l8, acc = sm_chunk(h0, cs, sbuf[us % NBUF], mbc, off, l8, acc)
                if cs == NC - 1:
                    finish(t0 + us, l8, acc)
            mb_next = colmax(m8)
        return mb, l8, acc, mb_next

    zero8 = jnp.zeros((8, TQ), F32)
    mb, l8, acc, mb_next = jax.lax.fori_loop(
        0, NT // TPI, attn_body, (zero8, zero8, jnp.zeros((DH, TQ), F32), zero8))
    off = (pl.program_id(0) >> 20) * 8
    for cs in range(NC - SK, NC):
        l8, acc = sm_chunk(H - 1, cs, sbuf[(NT - 2) % NBUF], mb, off, l8, acc)
    finish(NT - 2, l8, acc)
    l8, acc = None, None
    for cs in range(NC):
        l8, acc = sm_chunk(H - 1, cs, sbuf[(NT - 1) % NBUF], mb_next, off, l8, acc)
    finish(NT - 1, l8, acc)

    for cp in rest_all:
        cp.wait()

    def b_proj_a_out(r, carry):
        slot = r % 2

        @pl.when(r >= 2)
        def _():
            out_copy(slot, r - 2, 0).wait()

        rows = pl.ds(pl.multiple_of(r * TR, TR), TR)
        x = xb[rows, :]
        pkt = []
        for c in range(2):
            y = jnp.dot(x, wb[:, D + c * CW:D + (c + 1) * CW], preferred_element_type=F32)
            pk = _phi(y)
            zacc[:, c * CW:(c + 1) * CW] += jnp.sum(pk.reshape(TR // 8, 8, CW), axis=0)
            pkt.append(pk.T.astype(BF16))
        vs = []
        for c in range(2):
            y = jnp.dot(x, wb[:, 2 * D + c * CW:2 * D + (c + 1) * CW], preferred_element_type=F32)
            vs.append(y.astype(BF16))
        y = jnp.dot(ot[:, rows].T, woa[...], preferred_element_type=F32)
        stage[slot] = y.astype(BF16)
        for g in range(G):
            c, o = divmod(g * 128, CW)
            kvacc[g] += jnp.dot(pkt[c][o:o + 128, :], vs[c][:, o:o + 128], preferred_element_type=F32)
        for c in range(2):
            y = jnp.dot(x, wb[:, c * CW:(c + 1) * CW], preferred_element_type=F32)
            pq[rows, c * CW:(c + 1) * CW] = _phi(y).astype(BF16)
        out_copy(slot, r, 0).start()
        return carry

    jax.lax.fori_loop(0, NR, b_proj_a_out, 0)

    rh = jax.lax.broadcasted_iota(jnp.int32, (128, 128), 0) // DH
    ch = jax.lax.broadcasted_iota(jnp.int32, (128, 128), 1) // DH
    same_head = rh == ch
    z = jnp.sum(zacc[...], axis=0, keepdims=True)
    for g in range(G):
        sl = slice(g * 128, (g + 1) * 128)
        kvd = jnp.where(same_head, kvacc[g], 0.0).astype(BF16)
        mm[sl, :] = jnp.dot(kvd, wob[sl, :], preferred_element_type=F32).astype(BF16)
        zc = jnp.broadcast_to(z[:, sl], (128, 128)).T
        zdg = jnp.where(same_head, zc, 0.0).astype(BF16)
        for r in range(NR):
            rows = slice(r * TR, (r + 1) * TR)
            a = pq[rows, sl]
            den = jnp.dot(a, zdg, preferred_element_type=F32) + 1e-6
            an[rows, sl] = (a.astype(F32) * _recip(den)).astype(BF16)

    def outb_copy(n):
        r0, nr = OUTB[n]
        return pltpu.make_async_copy(
            stageb.at[pl.ds(r0, nr), :],
            out_hbm.at[pl.ds(r0, nr), pl.ds(D, D)],
            outb_sems.at[n])

    for n, (r0, nr) in enumerate(OUTB):
        for q0 in range(r0, r0 + nr, TR):
            q1 = min(q0 + TR, r0 + nr)
            y = jnp.dot(an[q0:q1, :], mm[...], preferred_element_type=F32)
            stageb[q0:q1, :] = y.astype(BF16)
        outb_copy(n).start()

    out_copy(0, NR - 2, 0).wait()
    out_copy(1, NR - 1, 0).wait()
    for n in range(len(OUTB)):
        outb_copy(n).wait()


OUTB = ((0, 1536), (1536, 256), (1792, 256))


@jax.jit
def pallas_concat_heads__mha_block__linear_attn_block__prompt_kernel(
    A_x: jax.Array,
    A_wqkv: jax.Array,
    A_wo: jax.Array,
    B_x: jax.Array,
    B_wqkv: jax.Array,
    B_wo: jax.Array,
):
    xa = A_x.reshape(S, D)
    xb = B_x.reshape(S, D)
    any_spec = pl.BlockSpec(memory_space=pl.ANY)
    out = pl.pallas_call(
        _kernel,
        out_shape=jax.ShapeDtypeStruct((S, 2 * D), BF16),
        in_specs=[any_spec] * 6,
        out_specs=any_spec,
        grid=(1,),
        scratch_shapes=[
            pltpu.VMEM((S, D), BF16),
            pltpu.VMEM((D, 3 * D), BF16),
            pltpu.VMEM((D, D), BF16),
            pltpu.VMEM((S, D), BF16),
            pltpu.VMEM((D, 3 * D), BF16),
            pltpu.VMEM((D, D), BF16),
            pltpu.VMEM((D // 2, S), U32),
            pltpu.VMEM((D // 2, S), U32),
            pltpu.VMEM((H, S // 2, DH), U32),
            pltpu.VMEM((S, TQ), F32),
            pltpu.VMEM((S, TQ), F32),
            pltpu.VMEM((S, TQ), F32),
            pltpu.VMEM((S, TQ), F32),
            pltpu.VMEM((D, S), BF16),
            pltpu.VMEM((S, D), BF16),
            pltpu.VMEM((G, 128, 128), F32),
            pltpu.VMEM((8, D), F32),
            pltpu.VMEM((D, D), BF16),
            pltpu.VMEM((S, D), BF16),
            pltpu.VMEM((2, TR, D), BF16),
            pltpu.VMEM((S, D), BF16),
            pltpu.SemaphoreType.DMA((S // XP,)),
            pltpu.SemaphoreType.DMA((3 * D // WP,)),
            pltpu.SemaphoreType.DMA((4,)),
            pltpu.SemaphoreType.DMA((2,)),
            pltpu.SemaphoreType.DMA((len(OUTB),)),
        ],
        compiler_params=pltpu.CompilerParams(vmem_limit_bytes=120 * 1024 * 1024),
    )(xa, A_wqkv, A_wo, xb, B_wqkv, B_wo)
    return out.reshape(1, S, 2 * D)
```

```python
import math

import jax
import jax.numpy as jnp
import jax.experimental.pallas as pl
import jax.experimental.pallas.tpu as pltpu

S = 2048
D = 1024
H = 32
DH = 32
G = 8

TR = 512
NR = S // TR
CW = 512
XP = 256
WP = 256
TQ = 512
NQ = S // TQ
CK = 128
NC = S // CK
NT = H * NQ
TPI = 8
NBUF = 4
SK = 1
LAG = 3

F32 = jnp.float32
BF16 = jnp.bfloat16
U32 = jnp.uint32

QSCALE = (DH ** -0.5) * math.log2(math.e)


def _tie(x, dep):
    b = jax.lax.bitcast_convert_type(dep, jnp.int32)
    return jnp.where((b | 1) == 0, jnp.zeros_like(x), x)


def _phi(t):
    return jnp.where(t > 0, t + 1.0, jnp.exp(jnp.minimum(t, 0.0))) + 1e-6


def _pack(x):
    return pltpu.bitcast(x.astype(BF16), U32)


def _unpack(x):
    return pltpu.bitcast(x, BF16)


def _recip(x):
    r = pl.reciprocal(x, approx=True)
    return r * (2.0 - x * r)


def _kernel(xa_hbm, wa_hbm, woa_hbm, xb_hbm, wb_hbm, wob_hbm, out_hbm,
            xa, wa, woa, xb, wb, wob,
            qt, vt, kh, sb0, sb1, sb2, sb3, ot,
            tacc, zacc, mm, an,
            stage, stageb, xa_sems, wa_sems, in_sems, out_sems, outb_sems):
    def xa_copy(p):
        rows = pl.ds(p * XP, XP)
        return pltpu.make_async_copy(xa_hbm.at[rows, :], xa.at[rows, :], xa_sems.at[p])

    def wa_copy(p):
        cols = pl.ds(p * WP, WP)
        return pltpu.make_async_copy(wa_hbm.at[:, cols], wa.at[:, cols], wa_sems.at[p])

    rest = []
    rest_all = []
    for b, (src, dst, nrows) in enumerate(
            ((woa_hbm, woa, 512), (wb_hbm, wb, 176), (xb_hbm, xb, 512), (wob_hbm, wob, 512))):
        n = src.shape[0]
        r0 = 0
        while r0 < n:
            nr = min(nrows, n - r0)
            rest.append(pltpu.make_async_copy(src.at[pl.ds(r0, nr), :], dst.at[pl.ds(r0, nr), :],
                                              in_sems.at[b]))
            r0 += nr
        rest_all.append(pltpu.make_async_copy(src, dst, in_sems.at[b]))

    def out_copy(slot, r, col):
        return pltpu.make_async_copy(
            stage.at[slot],
            out_hbm.at[pl.ds(r * TR, TR), pl.ds(col * D, D)],
            out_sems.at[slot])

    def a_proj_mm(r0, nr, c0, nc):
        static = isinstance(r0, int)
        rows = pl.ds(r0 if static else pl.multiple_of(r0, nr), nr)
        return jnp.dot(xa[rows, :], wa[:, c0:c0 + nc], preferred_element_type=F32), (r0, nr, c0, nc)

    def a_proj_epi(yy):
        y, (r0, nr, c0, nc) = yy
        static = isinstance(r0, int)
        rows = pl.ds(r0 if static else pl.multiple_of(r0, nr), nr)
        rows2 = pl.ds(r0 // 2 if static else pl.multiple_of(r0 // 2, nr // 2), nr // 2)
        f0 = c0 % D
        if c0 < D:
            qt[f0 // 2:(f0 + nc) // 2, rows] = _pack((y * QSCALE).T)
        elif c0 < 2 * D:
            for hh in range(nc // DH):
                kh[f0 // DH + hh, rows2, :] = _pack(y[:, hh * DH:(hh + 1) * DH])
        else:
            vt[f0 // 2:(f0 + nc) // 2, rows] = _pack(y.T)

    def a_proj_piece(*a):
        a_proj_epi(a_proj_mm(*a))

    xa_copy(0).start()
    wa_copy(0).start()
    sb2[...] = jnp.zeros_like(sb2)
    sb3[...] = jnp.zeros_like(sb3)
    zacc[...] = jnp.zeros_like(zacc)
    tacc[...] = jnp.zeros_like(tacc)
    xa_copy(0).wait()
    wa_copy(1).start()
    wa_copy(0).wait()
    xa_copy(1).start()
    y = a_proj_mm(0, 256, 0, 256)
    wa_copy(1).wait()
    wa_copy(2).start()
    wa_copy(3).start()
    a_proj_epi(y)
    y = a_proj_mm(0, 256, 256, 256)
    xa_copy(1).wait()
    wa_copy(4).start()
    a_proj_epi(y)
    y = a_proj_mm(256, 256, 0, 512)
    wa_copy(2).wait()
    wa_copy(3).wait()
    for p in (5, 6, 7):
        wa_copy(p).start()
    a_proj_epi(y)
    y = a_proj_mm(0, 512, 512, 512)
    for p in (4, 5, 6, 7):
        wa_copy(p).wait()
    for p in (8, 9, 10, 11):
        wa_copy(p).start()
    a_proj_epi(y)
    a_proj_piece(0, 512, 1024, 512)
    y = a_proj_mm(0, 512, 1536, 512)
    for p in (8, 9, 10, 11):
        wa_copy(p).wait()
    xa_copy(2).start()
    xa_copy(3).start()
    a_proj_epi(y)
    a_proj_piece(0, 512, 2048, 512)
    a_proj_piece(0, 512, 2560, 512)

    def a_proj(r, carry):
        xa_copy(2 * r).wait()
        xa_copy(2 * r + 1).wait()

        @pl.when(r + 1 < NR)
        def _():
            xa_copy(2 * r + 2).start()
            xa_copy(2 * r + 3).start()

        for c in (0, 1, 4, 5, 2, 3):
            a_proj_piece(r * TR, TR, c * CW, CW)
        return carry

    jax.lax.fori_loop(1, NR, a_proj, 0)

    sbuf = [sb0, sb1, sb2, sb3]

    def hj(t):
        return t // NQ, t % NQ

    def load_q(t):
        h1, j1 = hj(t)
        q = qt[pl.ds(pl.multiple_of(h1 * (DH // 2), DH // 2), DH // 2),
               pl.ds(pl.multiple_of(j1 * TQ, TQ), TQ)]
        return h1, _unpack(q)

    def qk_chunk(h1, q, c, s_w, m8):
        k = _unpack(kh[h1, c * (CK // 2):(c + 1) * (CK // 2), :])
        s = jnp.dot(k, q, preferred_element_type=F32)
        s_w[c * CK:(c + 1) * CK, :] = s
        s3 = s.reshape(CK // 8, 8, TQ)
        for r in range(CK // 8):
            m8 = s3[r] if m8 is None else jnp.maximum(m8, s3[r])
        return m8

    def sm_chunk(h0, c, s_r, mbc, off, l8, acc):
        sv = s_r[pl.ds(pl.multiple_of(off + c * CK, 8), CK), :].reshape(CK // 8, 8, TQ)
        ps = [None] * (CK // 8)
        lt = None
        for r in reversed(range(CK // 8)):
            x = jnp.exp2(sv[r] - mbc)
            ps[r] = x
            lt = x if lt is None else lt + x
        l8 = lt if l8 is None else l8 + lt
        p = jnp.concatenate(ps, axis=0).astype(BF16)
        v = _unpack(vt[pl.ds(pl.multiple_of(h0 * (DH // 2), DH // 2), DH // 2), c * CK:(c + 1) * CK])
        o = jnp.dot(v, p, preferred_element_type=F32)
        acc = o if acc is None else acc + o
        return l8, acc

    def colmax(m8):
        return jnp.broadcast_to(jnp.max(m8, axis=0, keepdims=True), (8, TQ))

    def finish(t, l8, acc):
        h0, j0 = hj(jnp.maximum(t, 0))
        l = jnp.sum(l8, axis=0, keepdims=True)
        ot[pl.ds(pl.multiple_of(h0 * DH, DH), DH), pl.ds(pl.multiple_of(j0 * TQ, TQ), TQ)] = (
            acc * _recip(l)).astype(BF16)

    def attn_body(i, carry):
        mb, l8, acc, mb_next = carry
        for n, cp in enumerate(rest):
            @pl.when(i == n + 1)
            def _():
                cp.start()
        t0 = i * TPI
        off = (i >> 20) * 8
        hist = []
        h0, _ = hj(jnp.maximum(t0 - 2, 0))
        for u in range(TPI):
            h1, q = load_q(t0 + u)
            m8 = None
            for c in range(NC):
                m8 = qk_chunk(h1, q, c, sbuf[u % NBUF], m8)
                hist.append(m8)
                us = u - 1 if c >= SK else u - 2
                cs = (c - SK) % NC
                if cs == 0:
                    h0, _ = hj(jnp.maximum(t0 + us, 0))
                    mb, l8, acc = mb_next, None, None
                k = len(hist) - 1 - LAG
                mbc = _tie(mb, hist[k]) if k >= 0 else mb
                l8, acc = sm_chunk(h0, cs, sbuf[us % NBUF], mbc, off, l8, acc)
                if cs == NC - 1:
                    finish(t0 + us, l8, acc)
            mb_next = colmax(m8)
        return mb, l8, acc, mb_next

    zero8 = jnp.zeros((8, TQ), F32)
    mb, l8, acc, mb_next = jax.lax.fori_loop(
        0, NT // TPI, attn_body, (zero8, zero8, jnp.zeros((DH, TQ), F32), zero8))
    off = (pl.program_id(0) >> 20) * 8
    for cs in range(NC - SK, NC):
        l8, acc = sm_chunk(H - 1, cs, sbuf[(NT - 2) % NBUF], mb, off, l8, acc)
    finish(NT - 2, l8, acc)
    l8, acc = None, None
    for cs in range(NC):
        l8, acc = sm_chunk(H - 1, cs, sbuf[(NT - 1) % NBUF], mb_next, off, l8, acc)
    finish(NT - 1, l8, acc)

    for cp in rest_all:
        cp.wait()

    def b_proj_a_out(r, carry):
        slot = r % 2

        @pl.when(r >= 2)
        def _():
            out_copy(slot, r - 2, 0).wait()

        rows = pl.ds(pl.multiple_of(r * TR, TR), TR)
        x = xb[rows, :]
        pkt = []
        for c in range(2):
            y = jnp.dot(x, wb[:, D + c * CW:D + (c + 1) * CW], preferred_element_type=F32)
            pk = _phi(y)
            zacc[:, c * CW:(c + 1) * CW] += jnp.sum(pk.reshape(TR // 8, 8, CW), axis=0)
            pkt.append(pk.T.astype(BF16))
        y = jnp.dot(ot[:, rows].T, woa[...], preferred_element_type=F32)
        stage[slot] = y.astype(BF16)
        for c in range(2):
            tacc[c * CW:(c + 1) * CW, :] += jnp.dot(pkt[c], x, preferred_element_type=F32)
        out_copy(slot, r, 0).start()
        return carry

    jax.lax.fori_loop(0, NR, b_proj_a_out, 0)

    rh = jax.lax.broadcasted_iota(jnp.int32, (128, 128), 0) // DH
    ch = jax.lax.broadcasted_iota(jnp.int32, (128, 128), 1) // DH
    same_head = rh == ch
    z = jnp.sum(zacc[...], axis=0, keepdims=True)
    zcol = []
    for g in range(G):
        sl = slice(g * 128, (g + 1) * 128)
        kv = jnp.dot(tacc[sl, :].astype(BF16), wb[:, 2 * D + g * 128:2 * D + (g + 1) * 128],
                     preferred_element_type=F32)
        kvd = jnp.where(same_head, kv, 0.0).astype(BF16)
        mm[sl, :] = jnp.dot(kvd, wob[sl, :], preferred_element_type=F32).astype(BF16)
        zcol.append(jnp.broadcast_to(z[:, sl], (128, 128)).T)

    def b_q(r):
        rows = slice(r * TR, (r + 1) * TR)
        x = xb[rows, :]
        for c in range(2):
            y = jnp.dot(x, wb[:, c * CW:(c + 1) * CW], preferred_element_type=F32)
            pqt = _phi(y).astype(BF16).T
            for gg in range(CW // 128):
                g = c * (CW // 128) + gg
                parts = []
                for hh in range(128 // DH):
                    f0 = gg * 128 + hh * DH
                    a = pqt[f0:f0 + DH, :].astype(F32)
                    zh = zcol[g][hh * DH:(hh + 1) * DH, :]
                    w = a * jnp.concatenate([zh] * (TR // 128), axis=1)
                    den = jnp.sum(w, axis=0, keepdims=True) + 1e-6
                    parts.append(a * _recip(den))
                an[rows, g * 128:(g + 1) * 128] = jnp.concatenate(parts, axis=0).T.astype(BF16)

    def b_o(r0, nr):
        y = jnp.dot(an[r0:r0 + nr, :], mm[...], preferred_element_type=F32)
        stageb[r0:r0 + nr, :] = y.astype(BF16)

    def outb_copy(n):
        r0, nr = OUTB[n]
        return pltpu.make_async_copy(
            stageb.at[pl.ds(r0, nr), :],
            out_hbm.at[pl.ds(r0, nr), pl.ds(D, D)],
            outb_sems.at[n])

    b_q(0)
    for n in range(len(OUTB)):
        if n + 1 < NR:
            b_q(n + 1)
        b_o(*OUTB[n])
        outb_copy(n).start()

    out_copy(0, NR - 2, 0).wait()
    out_copy(1, NR - 1, 0).wait()
    for n in range(len(OUTB)):
        outb_copy(n).wait()


OUTB = ((0, 512), (512, 512), (1024, 512), (1536, 256), (1792, 128), (1920, 128))


@jax.jit
def pallas_concat_heads__mha_block__linear_attn_block__prompt_kernel(
    A_x: jax.Array,
    A_wqkv: jax.Array,
    A_wo: jax.Array,
    B_x: jax.Array,
    B_wqkv: jax.Array,
    B_wo: jax.Array,
):
    xa = A_x.reshape(S, D)
    xb = B_x.reshape(S, D)
    any_spec = pl.BlockSpec(memory_space=pl.ANY)
    out = pl.pallas_call(
        _kernel,
        out_shape=jax.ShapeDtypeStruct((S, 2 * D), BF16),
        in_specs=[any_spec] * 6,
        out_specs=any_spec,
        grid=(1,),
        scratch_shapes=[
            pltpu.VMEM((S, D), BF16),
            pltpu.VMEM((D, 3 * D), BF16),
            pltpu.VMEM((D, D), BF16),
            pltpu.VMEM((S, D), BF16),
            pltpu.VMEM((D, 3 * D), BF16),
            pltpu.VMEM((D, D), BF16),
            pltpu.VMEM((D // 2, S), U32),
            pltpu.VMEM((D // 2, S), U32),
            pltpu.VMEM((H, S // 2, DH), U32),
            pltpu.VMEM((S, TQ), F32),
            pltpu.VMEM((S, TQ), F32),
            pltpu.VMEM((S, TQ), F32),
            pltpu.VMEM((S, TQ), F32),
            pltpu.VMEM((D, S), BF16),
            pltpu.VMEM((D, D), F32),
            pltpu.VMEM((8, D), F32),
            pltpu.VMEM((D, D), BF16),
            pltpu.VMEM((S, D), BF16),
            pltpu.VMEM((2, TR, D), BF16),
            pltpu.VMEM((S, D), BF16),
            pltpu.SemaphoreType.DMA((S // XP,)),
            pltpu.SemaphoreType.DMA((3 * D // WP,)),
            pltpu.SemaphoreType.DMA((4,)),
            pltpu.SemaphoreType.DMA((2,)),
            pltpu.SemaphoreType.DMA((len(OUTB),)),
        ],
        compiler_params=pltpu.CompilerParams(vmem_limit_bytes=120 * 1024 * 1024),
    )(xa, A_wqkv, A_wo, xb, B_wqkv, B_wo)
    return out.reshape(1, S, 2 * D)
```

```python
import math

import jax
import jax.numpy as jnp
import jax.experimental.pallas as pl
import jax.experimental.pallas.tpu as pltpu

S = 2048
D = 1024
H = 32
DH = 32
G = 8

TR = 512
NR = S // TR
CW = 512
XP = 256
WP = 256
QC = 128
TQ = 512
NQ = S // TQ
CK = 128
NC = S // CK
NT = H * NQ
TPI = 8
NBUF = 4
SK = 1
LAG = 3

F32 = jnp.float32
BF16 = jnp.bfloat16
U32 = jnp.uint32

QSCALE = (DH ** -0.5) * math.log2(math.e)


def _tie(x, dep):
    b = jax.lax.bitcast_convert_type(dep, jnp.int32)
    return jnp.where((b | 1) == 0, jnp.zeros_like(x), x)


def _phi(t):
    return jnp.where(t > 0, t + 1.0, jnp.exp(jnp.minimum(t, 0.0))) + 1e-6


def _pack(x):
    return pltpu.bitcast(x.astype(BF16), U32)


def _unpack(x):
    return pltpu.bitcast(x, BF16)


def _recip(x):
    r = pl.reciprocal(x, approx=True)
    return r * (2.0 - x * r)


def _kernel(xa_hbm, wa_hbm, woa_hbm, xb_hbm, wb_hbm, wob_hbm, out_hbm,
            xa, wa, woa, xb, wb, wob,
            qt, vt, kh, sb0, sb1, sb2, sb3, ot,
            tacc, zacc, mm, an,
            stage, stageb, xa_sems, wa_sems, in_sems, out_sems, outb_sems):
    def xa_copy(p):
        rows = pl.ds(p * XP, XP)
        return pltpu.make_async_copy(xa_hbm.at[rows, :], xa.at[rows, :], xa_sems.at[p])

    def wa_copy(p):
        cols = pl.ds(p * WP, WP)
        return pltpu.make_async_copy(wa_hbm.at[:, cols], wa.at[:, cols], wa_sems.at[p])

    rest = []
    rest_all = []
    for b, (src, dst, nrows) in enumerate(
            ((woa_hbm, woa, 512), (wb_hbm, wb, 176), (xb_hbm, xb, 512), (wob_hbm, wob, 512))):
        n = src.shape[0]
        r0 = 0
        while r0 < n:
            nr = min(nrows, n - r0)
            rest.append(pltpu.make_async_copy(src.at[pl.ds(r0, nr), :], dst.at[pl.ds(r0, nr), :],
                                              in_sems.at[b]))
            r0 += nr
        rest_all.append(pltpu.make_async_copy(src, dst, in_sems.at[b]))

    def out_copy(slot, r, col):
        return pltpu.make_async_copy(
            stage.at[slot],
            out_hbm.at[pl.ds(r * TR, TR), pl.ds(col * D, D)],
            out_sems.at[slot])

    def a_proj_mm(r0, nr, c0, nc):
        static = isinstance(r0, int)
        rows = pl.ds(r0 if static else pl.multiple_of(r0, nr), nr)
        return jnp.dot(xa[rows, :], wa[:, c0:c0 + nc], preferred_element_type=F32), (r0, nr, c0, nc)

    def a_proj_epi(yy):
        y, (r0, nr, c0, nc) = yy
        static = isinstance(r0, int)
        rows = pl.ds(r0 if static else pl.multiple_of(r0, nr), nr)
        rows2 = pl.ds(r0 // 2 if static else pl.multiple_of(r0 // 2, nr // 2), nr // 2)
        f0 = c0 % D
        if c0 < D:
            qt[f0 // 2:(f0 + nc) // 2, rows] = _pack((y * QSCALE).T)
        elif c0 < 2 * D:
            for hh in range(nc // DH):
                kh[f0 // DH + hh, rows2, :] = _pack(y[:, hh * DH:(hh + 1) * DH])
        else:
            vt[f0 // 2:(f0 + nc) // 2, rows] = _pack(y.T)

    def a_proj_piece(*a):
        a_proj_epi(a_proj_mm(*a))

    xa_copy(0).start()
    wa_copy(0).start()
    sb2[...] = jnp.zeros_like(sb2)
    sb3[...] = jnp.zeros_like(sb3)
    zacc[...] = jnp.zeros_like(zacc)
    tacc[...] = jnp.zeros_like(tacc)
    xa_copy(0).wait()
    wa_copy(1).start()
    wa_copy(0).wait()
    xa_copy(1).start()
    y = a_proj_mm(0, 256, 0, 256)
    wa_copy(1).wait()
    wa_copy(2).start()
    wa_copy(3).start()
    a_proj_epi(y)
    y = a_proj_mm(0, 256, 256, 256)
    xa_copy(1).wait()
    wa_copy(4).start()
    a_proj_epi(y)
    y = a_proj_mm(256, 256, 0, 512)
    wa_copy(2).wait()
    wa_copy(3).wait()
    for p in (5, 6, 7):
        wa_copy(p).start()
    a_proj_epi(y)
    y = a_proj_mm(0, 512, 512, 512)
    for p in (4, 5, 6, 7):
        wa_copy(p).wait()
    for p in (8, 9, 10, 11):
        wa_copy(p).start()
    a_proj_epi(y)
    a_proj_piece(0, 512, 1024, 512)
    y = a_proj_mm(0, 512, 1536, 512)
    for p in (8, 9, 10, 11):
        wa_copy(p).wait()
    xa_copy(2).start()
    xa_copy(3).start()
    a_proj_epi(y)
    a_proj_piece(0, 512, 2048, 512)
    a_proj_piece(0, 512, 2560, 512)

    def a_proj(r, carry):
        xa_copy(2 * r).wait()
        xa_copy(2 * r + 1).wait()

        @pl.when(r + 1 < NR)
        def _():
            xa_copy(2 * r + 2).start()
            xa_copy(2 * r + 3).start()

        for c in (0, 1, 4, 5, 2, 3):
            a_proj_piece(r * TR, TR, c * CW, CW)
        return carry

    jax.lax.fori_loop(1, NR, a_proj, 0)

    sbuf = [sb0, sb1, sb2, sb3]

    def hj(t):
        return t // NQ, t % NQ

    def load_q(t):
        h1, j1 = hj(t)
        q = qt[pl.ds(pl.multiple_of(h1 * (DH // 2), DH // 2), DH // 2),
               pl.ds(pl.multiple_of(j1 * TQ, TQ), TQ)]
        return h1, _unpack(q)

    def qk_chunk(h1, q, c, s_w, m8):
        k = _unpack(kh[h1, c * (CK // 2):(c + 1) * (CK // 2), :])
        s = jnp.dot(k, q, preferred_element_type=F32)
        s_w[c * CK:(c + 1) * CK, :] = s
        s3 = s.reshape(CK // 8, 8, TQ)
        for r in range(CK // 8):
            m8 = s3[r] if m8 is None else jnp.maximum(m8, s3[r])
        return m8

    def sm_chunk(h0, c, s_r, mbc, off, l8, acc):
        sv = s_r[pl.ds(pl.multiple_of(off + c * CK, 8), CK), :].reshape(CK // 8, 8, TQ)
        ps = [None] * (CK // 8)
        lt = None
        for r in reversed(range(CK // 8)):
            x = jnp.exp2(sv[r] - mbc)
            ps[r] = x
            lt = x if lt is None else lt + x
        l8 = lt if l8 is None else l8 + lt
        p = jnp.concatenate(ps, axis=0).astype(BF16)
        v = _unpack(vt[pl.ds(pl.multiple_of(h0 * (DH // 2), DH // 2), DH // 2), c * CK:(c + 1) * CK])
        o = jnp.dot(v, p, preferred_element_type=F32)
        acc = o if acc is None else acc + o
        return l8, acc

    def colmax(m8):
        return jnp.broadcast_to(jnp.max(m8, axis=0, keepdims=True), (8, TQ))

    def finish(t, l8, acc):
        h0, j0 = hj(jnp.maximum(t, 0))
        l = jnp.sum(l8, axis=0, keepdims=True)
        ot[pl.ds(pl.multiple_of(h0 * DH, DH), DH), pl.ds(pl.multiple_of(j0 * TQ, TQ), TQ)] = (
            acc * _recip(l)).astype(BF16)

    def attn_body(i, carry):
        mb, l8, acc, mb_next = carry
        for n, cp in enumerate(rest):
            @pl.when(i == n + 1)
            def _():
                cp.start()
        t0 = i * TPI
        off = (i >> 20) * 8
        hist = []
        h0, _ = hj(jnp.maximum(t0 - 2, 0))
        for u in range(TPI):
            h1, q = load_q(t0 + u)
            m8 = None
            for c in range(NC):
                m8 = qk_chunk(h1, q, c, sbuf[u % NBUF], m8)
                hist.append(m8)
                us = u - 1 if c >= SK else u - 2
                cs = (c - SK) % NC
                if cs == 0:
                    h0, _ = hj(jnp.maximum(t0 + us, 0))
                    mb, l8, acc = mb_next, None, None
                k = len(hist) - 1 - LAG
                mbc = _tie(mb, hist[k]) if k >= 0 else mb
                l8, acc = sm_chunk(h0, cs, sbuf[us % NBUF], mbc, off, l8, acc)
                if cs == NC - 1:
                    finish(t0 + us, l8, acc)
            mb_next = colmax(m8)
        return mb, l8, acc, mb_next

    zero8 = jnp.zeros((8, TQ), F32)
    mb, l8, acc, mb_next = jax.lax.fori_loop(
        0, NT // TPI, attn_body, (zero8, zero8, jnp.zeros((DH, TQ), F32), zero8))
    off = (pl.program_id(0) >> 20) * 8
    for cs in range(NC - SK, NC):
        l8, acc = sm_chunk(H - 1, cs, sbuf[(NT - 2) % NBUF], mb, off, l8, acc)
    finish(NT - 2, l8, acc)
    l8, acc = None, None
    for cs in range(NC):
        l8, acc = sm_chunk(H - 1, cs, sbuf[(NT - 1) % NBUF], mb_next, off, l8, acc)
    finish(NT - 1, l8, acc)

    for cp in rest_all:
        cp.wait()

    def b_proj_a_out(r, carry):
        slot = r % 2

        @pl.when(r >= 2)
        def _():
            out_copy(slot, r - 2, 0).wait()

        rows = pl.ds(pl.multiple_of(r * TR, TR), TR)
        x = xb[rows, :]
        pkt = []
        for c in range(2):
            y = jnp.dot(x, wb[:, D + c * CW:D + (c + 1) * CW], preferred_element_type=F32)
            pk = _phi(y)
            zacc[:, c * CW:(c + 1) * CW] += jnp.sum(pk.reshape(TR // 8, 8, CW), axis=0)
            pkt.append(pk.T.astype(BF16))
        y = jnp.dot(ot[:, rows].T, woa[...], preferred_element_type=F32)
        stage[slot] = y.astype(BF16)
        for c in range(2):
            tacc[c * CW:(c + 1) * CW, :] += jnp.dot(pkt[c], x, preferred_element_type=F32)
        out_copy(slot, r, 0).start()
        return carry

    jax.lax.fori_loop(0, NR, b_proj_a_out, 0)

    rh = jax.lax.broadcasted_iota(jnp.int32, (128, 128), 0) // DH
    ch = jax.lax.broadcasted_iota(jnp.int32, (128, 128), 1) // DH
    same_head = rh == ch
    z = jnp.sum(zacc[...], axis=0, keepdims=True)
    zcol = []
    kvd = []
    for g in range(G):
        sl = slice(g * 128, (g + 1) * 128)
        kv = jnp.dot(tacc[sl, :].astype(BF16), wb[:, 2 * D + g * 128:2 * D + (g + 1) * 128],
                     preferred_element_type=F32)
        kvd.append(jnp.where(same_head, kv, 0.0).astype(BF16))
        zcol.append(jnp.broadcast_to(z[:, sl], (128, 128)).T)

    def fold_m():
        for g in range(G):
            sl = slice(g * 128, (g + 1) * 128)
            mm[sl, :] = jnp.dot(kvd[g], wob[sl, :], preferred_element_type=F32).astype(BF16)

    def b_q(r):
        rows = slice(r * TR, (r + 1) * TR)
        x = xb[rows, :]
        for c in range(D // QC):
            y = jnp.dot(x, wb[:, c * QC:(c + 1) * QC], preferred_element_type=F32)
            pqt = _phi(y).astype(BF16).T
            for gg in range(QC // 128):
                g = c * (QC // 128) + gg
                parts = []
                for hh in range(128 // DH):
                    f0 = gg * 128 + hh * DH
                    a = pqt[f0:f0 + DH, :].astype(F32)
                    zh = zcol[g][hh * DH:(hh + 1) * DH, :]
                    w = a * jnp.concatenate([zh] * (TR // 128), axis=1)
                    den = jnp.sum(w, axis=0, keepdims=True) + 1e-6
                    parts.append(a * _recip(den))
                an[rows, g * 128:(g + 1) * 128] = jnp.concatenate(parts, axis=0).T.astype(BF16)

    def b_o(r0, nr):
        y = jnp.dot(an[r0:r0 + nr, :], mm[...], preferred_element_type=F32)
        stageb[r0:r0 + nr, :] = y.astype(BF16)

    def outb_copy(n):
        r0, nr = OUTB[n]
        return pltpu.make_async_copy(
            stageb.at[pl.ds(r0, nr), :],
            out_hbm.at[pl.ds(r0, nr), pl.ds(D, D)],
            outb_sems.at[n])

    b_q(0)
    fold_m()
    for n in range(len(OUTB)):
        if n + 1 < NR:
            b_q(n + 1)
        b_o(*OUTB[n])
        outb_copy(n).start()

    out_copy(0, NR - 2, 0).wait()
    out_copy(1, NR - 1, 0).wait()
    for n in range(len(OUTB)):
        outb_copy(n).wait()


OUTB = ((0, 512), (512, 512), (1024, 512), (1536, 256), (1792, 128), (1920, 128))


@jax.jit
def pallas_concat_heads__mha_block__linear_attn_block__prompt_kernel(
    A_x: jax.Array,
    A_wqkv: jax.Array,
    A_wo: jax.Array,
    B_x: jax.Array,
    B_wqkv: jax.Array,
    B_wo: jax.Array,
):
    xa = A_x.reshape(S, D)
    xb = B_x.reshape(S, D)
    any_spec = pl.BlockSpec(memory_space=pl.ANY)
    out = pl.pallas_call(
        _kernel,
        out_shape=jax.ShapeDtypeStruct((S, 2 * D), BF16),
        in_specs=[any_spec] * 6,
        out_specs=any_spec,
        grid=(1,),
        scratch_shapes=[
            pltpu.VMEM((S, D), BF16),
            pltpu.VMEM((D, 3 * D), BF16),
            pltpu.VMEM((D, D), BF16),
            pltpu.VMEM((S, D), BF16),
            pltpu.VMEM((D, 3 * D), BF16),
            pltpu.VMEM((D, D), BF16),
            pltpu.VMEM((D // 2, S), U32),
            pltpu.VMEM((D // 2, S), U32),
            pltpu.VMEM((H, S // 2, DH), U32),
            pltpu.VMEM((S, TQ), F32),
            pltpu.VMEM((S, TQ), F32),
            pltpu.VMEM((S, TQ), F32),
            pltpu.VMEM((S, TQ), F32),
            pltpu.VMEM((D, S), BF16),
            pltpu.VMEM((D, D), F32),
            pltpu.VMEM((8, D), F32),
            pltpu.VMEM((D, D), BF16),
            pltpu.VMEM((S, D), BF16),
            pltpu.VMEM((2, TR, D), BF16),
            pltpu.VMEM((S, D), BF16),
            pltpu.SemaphoreType.DMA((S // XP,)),
            pltpu.SemaphoreType.DMA((3 * D // WP,)),
            pltpu.SemaphoreType.DMA((4,)),
            pltpu.SemaphoreType.DMA((2,)),
            pltpu.SemaphoreType.DMA((len(OUTB),)),
        ],
        compiler_params=pltpu.CompilerParams(vmem_limit_bytes=120 * 1024 * 1024),
    )(xa, A_wqkv, A_wo, xb, B_wqkv, B_wo)
    return out.reshape(1, S, 2 * D)
```
